```python
import os as _os
_os.environ.setdefault("JAX_PLATFORMS", "cpu")
import jax
import jax.numpy as jnp

def _softmax(x, axis=-1):
    return jax.nn.softmax(x, axis=axis)
def _gelu(x):
    return jax.nn.gelu(x, approximate=True)
def _silu(x):
    return jax.nn.silu(x)
def _sigmoid(x):
    return jax.nn.sigmoid(x)
def _layernorm(x, axis=-1, eps=1e-5):
    m = jnp.mean(x, axis=axis, keepdims=True)
    v = jnp.var(x, axis=axis, keepdims=True)
    return (x - m) / jnp.sqrt(v + eps)
def _scatter_add(tgt, idx, src, axis=0):
    return tgt.at[idx].add(src)
def _segment_sum(src, seg, n):
    return jax.ops.segment_sum(src, seg, n)
class _Rng:
    def __init__(self, key):
        self._k = key
    def _next(self):
        self._k, sub = jax.random.split(self._k)
        return sub
    def normal(self, shape):
        return jax.random.normal(self._next(), shape, dtype=jnp.bfloat16)
    def randint(self, lo, hi, shape):
        return jax.random.randint(self._next(), shape, lo, hi, dtype=jnp.int32)
    def uniform(self, shape, lo=0.0, hi=1.0):
        return jax.random.uniform(self._next(), shape, jnp.bfloat16, lo, hi)
    def permutation(self, n):
        return jax.random.permutation(self._next(), n)


kernel_name = 'parallel_sum__softmax_full_mha__swiglu_ffn__prompt'

def setup_inputs():
    _rng = _Rng(jax.random.key(int.from_bytes(__import__("os").urandom(4), "little")))
    _w = (lambda a: (lambda t: t.astype(jnp.bfloat16) if jnp.issubdtype(t.dtype, jnp.floating) else t)(jnp.asarray(a)))
    def _A_setup():
        B, S, D = 1, 2048, 640
        return {
            "x": _w((lambda *s: _rng.normal(s) * 0.05)(B, S, D)),
            "wqkv": _w((lambda *s: _rng.normal(s) * 0.1)(D, 3 * D)),
            "wo": _w((lambda *s: _rng.normal(s) * 0.05)(D, D)),
        }
    _A_in = _A_setup()

    def _B_setup():
        B, S, D, F = 1, 2048, 640, 1536
        return {
            "x": _w((lambda *s: _rng.normal(s) * 0.05)(B, S, D)),
            "w_gate": _w((lambda *s: _rng.normal(s) * 0.05)(D, F)),
            "w_up": _w((lambda *s: _rng.normal(s) * 0.05)(D, F)),
            "w_down": _w((lambda *s: _rng.normal(s) * 0.05)(F, D)),
        }
    _B_in = _B_setup()

    return {
        "A_x": _A_in["x"],
        "A_wqkv": _A_in["wqkv"],
        "A_wo": _A_in["wo"],
        "B_x": _B_in["x"],
        "B_w_gate": _B_in["w_gate"],
        "B_w_up": _B_in["w_up"],
        "B_w_down": _B_in["w_down"],
    }

def reference(A_x, A_wqkv, A_wo, B_x, B_w_gate, B_w_up, B_w_down):
    def _A_ref(x, wqkv, wo):
        B, S, D = x.shape
        H = 32; Dh = D // H
        qkv = (lambda x, *d: x.transpose(*d))((x @ wqkv).reshape(B, S, 3, H, Dh), 2, 0, 3, 1, 4)
        q, k, v = qkv[0], qkv[1], qkv[2]
        scale = Dh ** -0.5
        scores = jnp.einsum("bhqd,bhkd->bhqk", q, k) * scale
        p = _softmax(scores, axis=-1)
        o = jnp.einsum("bhqk,bhkd->bhqd", p, v)
        return (lambda x, *d: x.transpose(*d))(o, 0, 2, 1, 3).reshape(B, S, D) @ wo

    def _B_ref(x, w_gate, w_up, w_down):
        g = _silu(x @ w_gate)
        u = x @ w_up
        return (g * u) @ w_down

    x = A_x
    xn = _layernorm(x, axis=-1)
    return x + _A_ref(xn, A_wqkv, A_wo) + _B_ref(xn, B_w_gate, B_w_up, B_w_down)
```

```python
import jax
import jax.numpy as jnp
import jax.experimental.pallas as pl
import jax.experimental.pallas.tpu as pltpu

S, D, F, H, DH = 2048, 640, 1536, 32, 20
TQ = 512
KC = 128
NC = S // KC
NT = S // TQ
U = 4
NP = H // U
NSTEP = NT * NP
W = 24
FC = 512
QSCALE = DH ** -0.5 * 1.4426950408889634
BF, F32 = jnp.bfloat16, jnp.float32


def _dot(a, b):
    return jax.lax.dot_general(a, b, (((1,), (0,)), ((), ())), preferred_element_type=F32)


def _kernel(x_hbm, wqkv_hbm, wo_hbm, wg_hbm, wu_hbm, wd_hbm, o_hbm,
            x_v, wqkv, wo, wg, wu, wd, xn_v, kh, qt, vt, ot,
            s_v, p_v, sems, osems):
    rows = lambda t: pl.ds(pl.multiple_of(t * TQ, TQ), TQ)
    x_cp = [pltpu.make_async_copy(x_hbm.at[pl.ds(t * TQ, TQ)], x_v.at[pl.ds(t * TQ, TQ)], sems.at[t])
            for t in range(NT)]
    w_cp = [pltpu.make_async_copy(s, d, sems.at[NT + i]) for i, (s, d) in enumerate(
        [(wqkv_hbm, wqkv), (wo_hbm, wo), (wg_hbm, wg), (wu_hbm, wu), (wd_hbm, wd)])]
    x_cp[0].start()
    w_cp[0].start()

    w_cp[0].wait()
    for c in x_cp[1:]:
        c.start()

    def proj(t, _):
        pltpu.make_async_copy(x_hbm.at[rows(t)], x_v.at[rows(t)], sems.at[t]).wait()
        x = x_v[rows(t), :].astype(F32)
        xc = x - jnp.mean(x, axis=-1, keepdims=True)
        var = jnp.mean(xc * xc, axis=-1, keepdims=True)
        xn = (xc * jax.lax.rsqrt(var + 1e-5)).astype(BF)
        xn_v[rows(t), :] = xn
        k = pltpu.bitcast(_dot(xn, wqkv[:, D:2 * D]).astype(BF), jnp.uint32)
        q = (_dot(xn, wqkv[:, 0:D]) * QSCALE).T
        v = _dot(xn, wqkv[:, 2 * D:3 * D]).T
        lane = jax.lax.broadcasted_iota(jnp.int32, (TQ // 2, 128), 1)
        row = jax.lax.broadcasted_iota(jnp.int32, (W, TQ), 0)
        zpad = jnp.zeros((32 - W, TQ), F32)
        for h in range(H):
            a = DH * h - 4 * (h % 2)
            g, o = a // 128, a % 128
            src = k[:, g * 128:(g + 1) * 128]
            if o + W > 128:
                src = jnp.where(lane >= o, src, k[:, (g + 1) * 128:(g + 2) * 128])
            if o:
                src = pltpu.roll(src, 128 - o, 1)
            kh[h, rows(t), :] = pltpu.bitcast(src, BF)[:, 0:32]
            mine = (row >= 4) if h % 2 else (row < DH)
            qt[h, :, rows(t)] = jnp.concatenate(
                [jnp.where(mine, q[a:a + W], 0.0), zpad], axis=0).astype(BF)
            vt[h, :, rows(t)] = jnp.where(mine, v[a:a + W], 1.0)
        return 0

    jax.lax.fori_loop(0, NT, proj, 0)
    for c in w_cp[1:]:
        c.start()

    def step(i, m8, do_a=True, do_b=True, do_c=True):
        m_out, on = [], []
        for u in range(U):
            if do_a:
                ia = i + 2
                ha = U * (ia % NP) + u
                q = qt[ha, :, rows(ia // NP)]
            if do_b:
                m = jnp.max(m8[u], axis=0, keepdims=True)
            if do_c:
                hc = U * (i % NP) + u
            mn = jnp.full((8, TQ), -jnp.inf, F32)
            acc = jnp.zeros((W, TQ), F32)
            for c in range(NC):
                ck = slice(c * KC, (c + 1) * KC)
                if do_c:
                    acc = acc + _dot(vt[hc, :, ck], p_v[u, ck, :])
                if do_b:
                    p_v[u, ck, :] = jnp.exp2(s_v[u, ck, :] - m).astype(BF)
                if do_a:
                    s = _dot(kh[ha, ck, :], q)
                    s_v[u, ck, :] = s
                    mn = jnp.maximum(mn, jnp.max(s.reshape(KC // 8, 8, TQ), axis=0))
            m_out.append(mn)
            if do_c:
                den = acc[0:1] if u % 2 else acc[DH:DH + 1]
                on.append(acc / den)
        if do_c:
            r8 = jax.lax.broadcasted_iota(jnp.int32, (8, TQ), 0)
            parts = []
            for e, o in zip(on[0::2], on[1::2]):
                parts += [e[0:16], jnp.where(r8 < 4, e[16:24], o[0:8]), o[8:24]]
            ot[pl.ds(pl.multiple_of((i % NP) * (U * DH), 8), U * DH), rows(i // NP)] = (
                jnp.concatenate(parts, axis=0))
        return tuple(m_out)

    m8 = step(-2, None, do_b=False, do_c=False)
    m8 = step(-1, m8, do_c=False)
    m8 = jax.lax.fori_loop(0, NSTEP - 2, step, m8)
    m8 = step(NSTEP - 2, m8, do_a=False)
    step(NSTEP - 1, m8, do_a=False, do_b=False)

    for c in w_cp[1:]:
        c.wait()

    def out_copy(t):
        return pltpu.make_async_copy(x_v.at[rows(t)], o_hbm.at[rows(t)], osems.at[t])

    def post(t, _):
        xn = xn_v[rows(t), :]
        acc = x_v[rows(t), :].astype(F32) + _dot(ot[:, rows(t)].T.astype(BF), wo[...])
        for f in range(F // FC):
            cf = slice(f * FC, (f + 1) * FC)
            g = _dot(xn, wg[:, cf])
            u = _dot(xn, wu[:, cf])
            acc = acc + _dot((g * jax.nn.sigmoid(g) * u).astype(BF), wd[cf, :])
        x_v[rows(t), :] = acc.astype(BF)
        out_copy(t).start()
        return 0

    jax.lax.fori_loop(0, NT, post, 0)
    for t in range(NT):
        out_copy(t).wait()


@jax.jit
def pallas_parallel_sum__softmax_full_mha__swiglu_ffn__prompt_kernel(
    A_x: jax.Array,
    A_wqkv: jax.Array,
    A_wo: jax.Array,
    B_x: jax.Array,
    B_w_gate: jax.Array,
    B_w_up: jax.Array,
    B_w_down: jax.Array,
):
    del B_x
    out = pl.pallas_call(
        _kernel,
        out_shape=jax.ShapeDtypeStruct((S, D), BF),
        in_specs=[pl.BlockSpec(memory_space=pl.ANY)] * 6,
        out_specs=pl.BlockSpec(memory_space=pl.ANY),
        scratch_shapes=[
            pltpu.VMEM((S, D), BF), pltpu.VMEM((D, 3 * D), BF), pltpu.VMEM((D, D), BF),
            pltpu.VMEM((D, F), BF), pltpu.VMEM((D, F), BF), pltpu.VMEM((F, D), BF),
            pltpu.VMEM((S, D), BF),
            pltpu.VMEM((H, S, 32), BF), pltpu.VMEM((H, 32, S), BF), pltpu.VMEM((H, W, S), F32),
            pltpu.VMEM((D, S), F32),
            pltpu.VMEM((U, S, TQ), F32),
            pltpu.VMEM((U, S, TQ), BF),
            pltpu.SemaphoreType.DMA((NT + 5,)), pltpu.SemaphoreType.DMA((NT,)),
        ],
        compiler_params=pltpu.CompilerParams(vmem_limit_bytes=120 * 1024 * 1024),
    )(A_x.reshape(S, D), A_wqkv, A_wo, B_w_gate, B_w_up, B_w_down)
    return out.reshape(A_x.shape)
```
